```python
import os as _os
_os.environ.setdefault("JAX_PLATFORMS", "cpu")
import jax
import jax.numpy as jnp

def _softmax(x, axis=-1):
    return jax.nn.softmax(x, axis=axis)
def _gelu(x):
    return jax.nn.gelu(x, approximate=True)
def _silu(x):
    return jax.nn.silu(x)
def _sigmoid(x):
    return jax.nn.sigmoid(x)
def _layernorm(x, axis=-1, eps=1e-5):
    m = jnp.mean(x, axis=axis, keepdims=True)
    v = jnp.var(x, axis=axis, keepdims=True)
    return (x - m) / jnp.sqrt(v + eps)
def _scatter_add(tgt, idx, src, axis=0):
    return tgt.at[idx].add(src)
def _segment_sum(src, seg, n):
    return jax.ops.segment_sum(src, seg, n)
class _Rng:
    def __init__(self, key):
        self._k = key
    def _next(self):
        self._k, sub = jax.random.split(self._k)
        return sub
    def normal(self, shape):
        return jax.random.normal(self._next(), shape, dtype=jnp.bfloat16)
    def randint(self, lo, hi, shape):
        return jax.random.randint(self._next(), shape, lo, hi, dtype=jnp.int32)
    def uniform(self, shape, lo=0.0, hi=1.0):
        return jax.random.uniform(self._next(), shape, jnp.bfloat16, lo, hi)
    def permutation(self, n):
        return jax.random.permutation(self._next(), n)


kernel_name = 'standalone__seq2seq_rnn_t_joint__speech'

def setup_inputs():
    _rng = _Rng(jax.random.key(int.from_bytes(__import__("os").urandom(4), "little")))
    _w = (lambda a: (lambda t: t.astype(jnp.bfloat16) if jnp.issubdtype(t.dtype, jnp.floating) else t)(jnp.asarray(a)))
    B, T, D, K = 2, 16000, 256, 31
    U = 8
    sc = (1.0 / (K * D)) ** 0.5
    sd = (1.0 / D) ** 0.5
    return {
        "x": _w((lambda *s: _rng.normal(s) * 0.2)(B, T, D) * 0.5),
        "w1": _w((lambda *s: _rng.normal(s) * 1.6)(K, D, D) * sc),
        "w2": _w((lambda *s: _rng.normal(s) * 1.6)(K, D, D) * sc),
        "g": _w((lambda *s: _rng.normal(s) * 1.6)(B, U, D) * 0.5),
        "w_f": _w((lambda *s: _rng.normal(s) * 1.6)(D, D) * sd),
        "w_g": _w((lambda *s: _rng.normal(s) * 1.6)(D, D) * sd),
        "w_o": _w((lambda *s: _rng.normal(s) * 1.6)(D, D) * sd),
    }

def reference(x, w1, w2, g, w_f, w_g, w_o):
    B, T, D = x.shape
    K = w1.shape[0]
    pad = K // 2
    xp = jnp.pad(x, ((0,0),(pad,pad),(0,0)))
    h = jnp.zeros_like(x)
    for i in range(K):
        h = h + jnp.einsum("btc,cd->btd", xp[:, i:i+T, :], w1[i])
    h = _gelu(h)[:, ::2, :]
    T1 = h.shape[1]
    hp = jnp.pad(h, ((0,0),(pad,pad),(0,0)))
    f = jnp.zeros_like(h)
    for i in range(K):
        f = f + jnp.einsum("btc,cd->btd", hp[:, i:i+T1, :], w2[i])
    f = _gelu(f)[:, ::2, :]
    fe = jnp.einsum("btd,de->bte", f, w_f)
    ge = jnp.einsum("bud,de->bue", g, w_g)
    j = jnp.tanh(fe[:, :, None, :] + ge[:, None, :, :])
    return jnp.einsum("btud,dv->btuv", j, w_o)
```

```python
import itertools
import math
import jax
import jax.numpy as jnp
import jax.experimental.pallas as pl
import jax.experimental.pallas.tpu as pltpu

B, T, D, K, U = 2, 16000, 256, 31, 8
T1, T2 = T // 2, T // 4
F32, BF16, U32 = jnp.float32, jnp.bfloat16, jnp.uint32
HOP = 17
MB = 240
NG = MB // 16
XROWS = 8192
KS = 4
NT = 5
UN = 4
LEAD = -600
JB = 8
JROWS = JB * HOP * U


class _Net:
    def __init__(self):
        self.nodes = []

    def _new(self, nd):
        self.nodes.append(nd)
        return (len(self.nodes) - 1, 1)

    def inp(self, i): return self._new(('in', i))
    def add(self, a, b): return self._new(('add', a[0], a[1], b[0], b[1]))
    def sub(self, a, b): return self.add(a, (b[0], -b[1]))
    def mul(self, a, c): return self._new(('mul', a[0], c * a[1]))


def _neg(a): return (a[0], -a[1])


def _tw(n, a, k, N):
    k %= N
    re, im = a
    if k == 0: return a
    if 4 * k == N: return (im, _neg(re))
    c, s = math.cos(2 * math.pi * k / N), -math.sin(2 * math.pi * k / N)
    if (8 * k) % N == 0:
        r = math.sqrt(0.5)
        sc, ss = round(c / r), round(s / r)
        t1 = n.add((re[0], re[1] * sc), (im[0], -im[1] * ss))
        t2 = n.add((re[0], re[1] * ss), (im[0], im[1] * sc))
        return (n.mul(t1, r), n.mul(t2, r))
    return (n.sub(n.mul(re, c), n.mul(im, s)), n.add(n.mul(re, s), n.mul(im, c)))


def _cfft(n, x):
    N = len(x)
    if N == 1: return x
    cadd = lambda a, b: (n.add(a[0], b[0]), n.add(a[1], b[1]))
    csub = lambda a, b: (n.sub(a[0], b[0]), n.sub(a[1], b[1]))
    if N == 2: return [cadd(x[0], x[1]), csub(x[0], x[1])]
    h, q = N // 2, N // 4
    s, d = [], []
    for i in range(h):
        s.append(cadd(x[i], x[i + h])); d.append(csub(x[i], x[i + h]))
    E = _cfft(n, s)
    o1, o3 = [], []
    for i in range(q):
        mi = (d[i + q][1], _neg(d[i + q][0]))
        o1.append(_tw(n, cadd(d[i], mi), i, N))
        o3.append(_tw(n, csub(d[i], mi), 3 * i, N))
    O1, O3 = _cfft(n, o1), _cfft(n, o3)
    X = [None] * N
    for m in range(h): X[2 * m] = E[m]
    for m in range(q): X[4 * m + 1], X[4 * m + 3] = O1[m], O3[m]
    return X


def _odd(n, d, N):
    q = N // 4
    C = _cfft(n, [_tw(n, (d(i), _neg(d(i + q))), i, N) for i in range(q)])
    out = {}
    for m in range(q):
        f = 4 * m + 1
        if f < N // 2: out[f] = C[m]
        else: out[N - f] = (C[m][0], _neg(C[m][1]))
    return out


def _rfft(n, x, top=False):
    N = len(x)
    if N == 2: return {0: (n.add(x[0], x[1]), None), 1: (n.sub(x[0], x[1]), None)}
    h = N // 2
    if top:
        s = [n.add(x[i], x[i + h]) for i in range(h)]
        d = lambda i: n.sub(x[i], x[i + h])
    else:
        s, dl = [], []
        for i in range(h):
            dl.append(n.sub(x[i], x[i + h])); s.append(n.add(x[i], x[i + h]))
        d = lambda i: dl[i]
    out = {2 * f: v for f, v in _rfft(n, s).items()}
    out.update(_odd(n, d, N))
    return out


_NET = _Net()
_X = _rfft(_NET, [_NET.inp(i) for i in range(32)], top=True)
_SLOT = [(_X[0][0], _X[16][0])] + [_X[f] for f in range(1, 16)]
_EVEN = [0, 8, 4, 12, 2, 14, 10, 6]
_ODD = [1, 15, 9, 7, 5, 11, 13, 3]


def _sadd(a, b):
    if a is None: return b
    if b is None: return a
    if a[1] == b[1]: return (a[0] + b[0], a[1])
    if a[1] > 0: return (a[0] - b[0], 1)
    return (b[0] - a[0], 1)


def _sg(v, s): return None if v is None else (v[0], v[1] * s)
def _pos(v): return v[0] if v[1] > 0 else -v[0]


def _forward(get_in, slots, emit):
    nodes = _NET.nodes
    need, st = set(), [c[0] for k in slots for c in _SLOT[k]]
    while st:
        i = st.pop()
        if i not in need:
            need.add(i)
            nd = nodes[i]
            if nd[0] == 'add': st += [nd[1], nd[3]]
            elif nd[0] == 'mul': st.append(nd[1])
    memo = {}

    def val(i):
        if i not in memo:
            v = get_in(nodes[i][1])
            memo[i] = None if v is None else (v, 1)
        return memo[i]
    pending = list(slots)
    for i in sorted(need):
        nd = nodes[i]
        if i % 8 == 0: yield 20
        if nd[0] == 'add':
            memo[i] = _sadd(_sg(val(nd[1]), nd[2]), _sg(val(nd[3]), nd[4]))
        elif nd[0] == 'mul':
            v = val(nd[1])
            memo[i] = None if v is None else (v[0] * (nd[2] * v[1]), 1)
        for k in list(pending):
            re, im = _SLOT[k]
            if re[0] in memo and im[0] in memo:
                pending.remove(k)
                emit(k, _sg(memo[re[0]], re[1]), _sg(memo[im[0]], im[1]))


def _adjoint(get_y):
    nodes = _NET.nodes
    live = [False] * len(nodes)
    for i, nd in enumerate(nodes):
        live[i] = nd[1] < HOP if nd[0] == 'in' else (live[nd[1]] or (nd[0] == 'add' and live[nd[3]]))
    seed = {}
    for k in range(16):
        for c in range(2):
            seed.setdefault(_SLOT[k][c][0], []).append((k, c, _SLOT[k][c][1]))
    bar = {}
    for i in range(len(nodes) - 1, -1, -1):
        nd = nodes[i]
        for k, c, s in seed.get(i, ()):
            bar[i] = _sadd(bar.get(i), (get_y(k, c), s))
        if nd[0] == 'in' or not live[i]: continue
        if i % 16 == 0: yield 15
        v = bar.pop(i)
        if nd[0] == 'add':
            for j, s in ((nd[1], nd[2]), (nd[3], nd[4])):
                if live[j]: bar[j] = _sadd(bar.get(j), _sg(v, s))
        else:
            bar[nd[1]] = _sadd(bar.get(nd[1]), (v[0] * (nd[2] * v[1]), 1))
    return [bar[i] for i in range(HOP)]


_SIGN = {}
for _sl in (_EVEN, _ODD):
    list(_forward(lambda i: 1.0, _sl, lambda k, re, im: _SIGN.__setitem__(k, (re[1], im[1]))))


def _gelu(v):
    x, s = v
    x = x * (0.5 * s)
    return x + x * jnp.tanh(x * (2 * 0.7978845608028654 + (8 * 0.7978845608028654 * 0.044715) * (x * x)))


def _lo(u): return pltpu.bitcast(u << 16, F32)
def _hi(u): return pltpu.bitcast(u & jnp.uint32(0xFFFF0000), F32)


def _kernel(x_hbm, w1_hbm, w2_hbm, g_ref, wf_ref, wg_ref, wo_ref, o_hbm,
            xb, hb, wr1, wr2, ws1, ws2, sp0, sp1, y0, y1, fe0, fe1, ob, xsem, wsem, osem):
    xu = xb.bitcast(U32)
    hu = hb.bitcast(U32)
    xcut = ((0, 8192), (8192, T - 8192))

    def xcopy(bt, ch):
        r, n = xcut[ch]
        return [pltpu.make_async_copy(x_hbm.at[bt, pl.ds(r, n), pl.ds(128 * hf, 128)],
                                      xb.at[bt, hf, pl.ds(48 + r, n), :], xsem.at[4 * bt + 2 * ch + hf]) for hf in range(2)]
    wcopy = [pltpu.make_async_copy(w1_hbm, wr1, wsem.at[0]), pltpu.make_async_copy(w2_hbm, wr2, wsem.at[1])]

    def start(cs):
        for c in cs: c.start()

    def wait(cs):
        for c in cs: c.wait()

    start(wcopy[:1])
    start(xcopy(0, 0))
    xb[:, :, 0:48, :] = jnp.zeros((B, 2, 48, 128), BF16)
    xb[:, :, 48 + T:, :] = jnp.zeros((B, 2, 2 * XROWS + 16 - 48 - T, 128), BF16)
    hb[:, :, :, 2 * MB:, :] = jnp.zeros((B, 2, HOP, 32, 128), BF16)

    def wfft(w_ref, wsp, g):
        r = pl.multiple_of(g * 16, 16)
        for par in range(2):
            for hf in range(2):
                def get(j):
                    k = 2 * j - 1 + par
                    if j >= 16 or k < 0: return None
                    return w_ref[k, pl.ds(r, 16), 128 * hf:128 * hf + 128].astype(F32) * (1.0 / 16)

                def emit(k, re, im):
                    a, b = _SIGN[k]
                    if k == 0:
                        ws = (jnp.zeros((16, 128), F32), re[0] * (0.5 * re[1] * a), im[0] * (-0.5 * im[1] * b))
                    else:
                        vr, vi = re, _sg(im, -1)
                        ws = (_pos(_sg(vr, a)), _pos(_sg(_sadd(vi, _sg(vr, -1)), a)), _pos(_sg(_sadd(vr, vi), b)))
                    for c in range(3):
                        wsp[k, c, hf, pl.ds(256 * par + r, 16), :] = ws[c].astype(BF16)
                yield from _forward(get, _EVEN + _ODD, emit)

    def emit_spec(sp, r, col):
        def emit(k, re, im):
            sm = re[0] if k == 0 else (re[0] + im[0] if re[1] == im[1] else re[0] - im[0])
            for c, v in enumerate((sm, re[0], im[0])):
                sp[k, c, col, pl.ds(r, 16), :] = v.astype(BF16)
        return emit

    def fwd1(bt, ch, sp, g):
        r = pl.multiple_of(g * 16, 16)
        base = pl.multiple_of((ch * MB + r) * HOP, 16)
        for hf in range(2):
            xv = xu.at[bt, hf, pl.ds(base, 288), :]
            for par in range(2):
                for sl in (_EVEN, _ODD):
                    get = lambda n: (_lo, _hi)[par](xv[pl.ds(n, 16, stride=HOP), :])
                    yield from _forward(get, sl, emit_spec(sp, r, 2 * par + hf))

    def fwd2(bt, sp, g):
        r = pl.multiple_of(g * 16, 16)
        for hf in range(2):
            hv = hu.at[bt, hf, :, pl.ds(r, 24), :]
            for par in range(2):
                for sl in (_EVEN, _ODD):
                    def get(n):
                        blk, q = divmod(2 * n + par, HOP)
                        return (_lo, _hi)[blk % 2](hv[q, pl.ds(blk // 2, 16), :])
                    yield from _forward(get, sl, emit_spec(sp, r, 2 * par + hf))

    def mm(wsp, sp, yb, k, VT):
        ys = y1 if yb is y0 else y0

        def d(c, n):
            acc = None
            for i in range(0, 4, KS):
                lhs = jnp.concatenate([pltpu.bitcast(sp.bitcast(U32)[k, c, i + j], BF16) for j in range(KS)], axis=1)
                p = jnp.dot(lhs, pltpu.bitcast(wsp.bitcast(U32)[k, c, n, 64 * i:64 * (i + KS), :], BF16), preferred_element_type=F32)
                acc = p if acc is None else acc + p
                for t in range(NT):
                    z = jnp.maximum(k - 16, 0)
                    tk = p[t * MB // NT:t * MB // NT + 8]
                    z8 = pl.multiple_of(z * 8, 8)
                    ys[z + 16, z, pl.ds(z8, 8), 0:128] = tk
                    xu[z, z, pl.ds(z8 + XROWS, 8), :] = pltpu.bitcast(tk, U32)
                    hu[z, z, z, pl.ds(z8 + MB + 8, 8), :] = pltpu.bitcast(tk, U32)
                    yield VT * KS / 24 / NT
            return acc
        for n in range(2):
            k1 = yield from d(0, n)
            yb[k, 0, :, 128 * n:128 * n + 128] = k1 - (yield from d(2, n))
            yb[k, 1, :, 128 * n:128 * n + 128] = k1 + (yield from d(1, n))

    def inv(yb, r, hf, out):
        halves = []
        for a in range(2):
            get = lambda k, c: yb[k, 1 - c if k == 0 else c, pl.ds(r + 8 * a, 8), 128 * hf:128 * hf + 128]
            halves.append([])
            for v in (yield from _adjoint(get)):
                halves[a].append(_gelu(v))
                yield 10
        out[:] = [jnp.concatenate([halves[0][q], halves[1][q]], axis=0) for q in range(HOP)]

    def inv1(bt, ch, yb, g):
        r = pl.multiple_of(g * 16, 16)
        t = (ch * MB + r + jax.lax.broadcasted_iota(jnp.int32, (16, 128), 0)) * HOP - 16
        ok = {q: (t + q >= 0) & (t + q < T1) for q in (0, 9, 16)}
        for hf in range(2):
            out = []
            yield from inv(yb, r, hf, out)
            for q, v in enumerate(out):
                m = ok[0 if q < 9 else 9 if q < 16 else 16]
                hb[bt, hf, q, pl.ds(ch * MB + r, 16), :] = jnp.where(m, v, 0.0).astype(BF16)

    def inv2(yb, fe, g):
        r = pl.multiple_of(g * 16, 16)
        f = []
        for hf in range(2):
            out = []
            yield from inv(yb, r, hf, out)
            f.append(jnp.concatenate(out, axis=0).astype(BF16))
        f = jnp.concatenate(f, axis=1)
        e = jnp.dot(f, wf_ref[...], preferred_element_type=F32)
        for q in range(HOP):
            fe[q, pl.ds(r, 16), :] = e[16 * q:16 * q + 16]

    def ocopy(bt, i, s):
        n = JROWS if i is not None else T2 * U - (MB // JB - 1) * JROWS
        r = pl.multiple_of(i * JROWS, 16) if i is not None else (MB // JB - 1) * JROWS
        return pltpu.make_async_copy(ob.at[s, pl.ds(0, n), :], o_hbm.at[bt, pl.ds(r, n), :], osem.at[s])

    def jtile(fe, ge, i, s):
        r = pl.multiple_of(i * JB, JB)
        h = JB // 2
        for p in range(2):
            js = [jnp.tanh(fe[q, pl.ds(r + b, 1), :] + ge) for b in range(p * h, p * h + h) for q in range(HOP)]
            j = jnp.concatenate(js, axis=0).astype(BF16)
            ob[s, pl.ds(p * JROWS // 2, JROWS // 2), :] = jnp.dot(j, wo_ref[...], preferred_element_type=F32).astype(BF16)
            yield 300

    def joint(bt, fe, other):
        ge = jnp.dot(g_ref[bt], wg_ref[...], preferred_element_type=F32)
        nt = MB // JB // 2

        def body(i):
            s = 2 * (i % 2)

            @pl.when(i >= 2)
            def _():
                ocopy(bt, 0, s).wait()
                ocopy(bt, 0, s + 1).wait()
            weave(itertools.chain(jtile(fe, ge, 2 * i, s), jtile(fe, ge, 2 * i + 1, s + 1)), other(i))
            ocopy(bt, 2 * i, s).start()

            @pl.when(i < nt - 1)
            def _():
                ocopy(bt, 2 * i + 1, s + 1).start()
        loop(nt, body)
        s = 2 * ((nt - 1) % 2)
        ocopy(bt, None, s + 1).start()
        wait([ocopy(bt, 0, 2 - s), ocopy(bt, 0, 3 - s), ocopy(bt, 0, s), ocopy(bt, None, s + 1)])

    def loop(n, f):
        def body(i, _):
            f(i)
            return 0
        jax.lax.fori_loop(0, n, body, 0)

    def weave(a, b):
        ia, ib = 0, LEAD
        while a or b:
            if a and (not b or ia <= ib):
                c = next(a, None)
                if c is None: a = None
                else: ia += c
            else:
                c = next(b, None)
                if c is None: b = None
                else: ib += c

    run = lambda gen: weave(gen, None)

    def step(name, m, *rest):
        def body(i):
            ks = [UN * i + u for u in range(UN)]
            weave(itertools.chain(*[mm(*m, k, 3600 if len(rest) > 1 else 1450) for k in ks]),
                  itertools.chain(*[f(jnp.minimum(k, NG - 1), k) for k in ks for f in rest]))
        with jax.named_scope(name):
            loop(16 // UN, body)

    wait(wcopy[:1])
    start(wcopy[1:])
    start(xcopy(0, 1))
    with jax.named_scope("wfft"):
        loop(16, lambda g: run(wfft(wr1, ws1, g)))
    wait(xcopy(0, 0))
    start(xcopy(1, 0))
    start(xcopy(1, 1))
    with jax.named_scope("s0"):
        loop(NG, lambda g: run(fwd1(0, 0, sp0, g)))
    wait(wcopy[1:])
    wait(xcopy(0, 1))
    step("s1", (ws1, sp0, y0), lambda g, k: fwd1(0, 1, sp1, g), lambda g, k: wfft(wr2, ws2, k))
    wait(xcopy(1, 0))
    step("s2", (ws1, sp1, y1), lambda g, k: inv1(0, 0, y0, g), lambda g, k: fwd1(1, 0, sp0, g))
    wait(xcopy(1, 1))
    step("s3", (ws1, sp0, y0), lambda g, k: inv1(0, 1, y1, g), lambda g, k: fwd1(1, 1, sp1, g))
    step("s4", (ws1, sp1, y1), lambda g, k: inv1(1, 0, y0, g), lambda g, k: fwd2(0, sp0, g))
    step("s5", (ws2, sp0, y0), lambda g, k: inv1(1, 1, y1, g), lambda g, k: fwd2(1, sp1, g))
    step("s6", (ws2, sp1, y1), lambda g, k: inv2(y0, fe0, g))
    with jax.named_scope("s7"):
        joint(0, fe0, lambda g: inv2(y1, fe1, g))
    with jax.named_scope("s8"):
        joint(1, fe1, lambda g: None)


@jax.jit
def pallas_standalone__seq2seq_rnn_t_joint__speech_kernel(x, w1, w2, g, w_f, w_g, w_o):
    vm = pl.BlockSpec(memory_space=pltpu.VMEM)
    hbm = pl.BlockSpec(memory_space=pl.ANY)
    two = lambda s, d: [pltpu.VMEM(s, d), pltpu.VMEM(s, d)]
    out = pl.pallas_call(
        _kernel,
        in_specs=[hbm] * 3 + [vm] * 4,
        out_specs=hbm,
        out_shape=jax.ShapeDtypeStruct((B, T2 * U, D), BF16),
        scratch_shapes=[
            pltpu.VMEM((B, 2, 2 * XROWS + 16, 128), BF16),
            pltpu.VMEM((B, 2, HOP, 2 * MB + 32, 128), BF16),
            *two((K, D, D), BF16),
            *two((16, 3, 2, 512, 128), BF16),
            *two((16, 3, 4, MB, 128), BF16),
            *two((17, 2, MB, 256), F32),
            *two((HOP, MB, 256), F32),
            pltpu.VMEM((4, JROWS, D), BF16),
            pltpu.SemaphoreType.DMA((8,)),
            pltpu.SemaphoreType.DMA((2,)),
            pltpu.SemaphoreType.DMA((4,)),
        ],
        compiler_params=pltpu.CompilerParams(vmem_limit_bytes=126 * 1024 * 1024),
    )(x, w1, w2, g, w_f, w_g, w_o)
    return out.reshape(B, T2, U, D)
```
